```python
import os as _os
_os.environ.setdefault("JAX_PLATFORMS", "cpu")
import jax
import jax.numpy as jnp

def _softmax(x, axis=-1):
    return jax.nn.softmax(x, axis=axis)
def _gelu(x):
    return jax.nn.gelu(x, approximate=True)
def _silu(x):
    return jax.nn.silu(x)
def _sigmoid(x):
    return jax.nn.sigmoid(x)
def _layernorm(x, axis=-1, eps=1e-5):
    m = jnp.mean(x, axis=axis, keepdims=True)
    v = jnp.var(x, axis=axis, keepdims=True)
    return (x - m) / jnp.sqrt(v + eps)
def _scatter_add(tgt, idx, src, axis=0):
    return tgt.at[idx].add(src)
def _segment_sum(src, seg, n):
    return jax.ops.segment_sum(src, seg, n)
class _Rng:
    def __init__(self, key):
        self._k = key
    def _next(self):
        self._k, sub = jax.random.split(self._k)
        return sub
    def normal(self, shape):
        return jax.random.normal(self._next(), shape, dtype=jnp.bfloat16)
    def randint(self, lo, hi, shape):
        return jax.random.randint(self._next(), shape, lo, hi, dtype=jnp.int32)
    def uniform(self, shape, lo=0.0, hi=1.0):
        return jax.random.uniform(self._next(), shape, jnp.bfloat16, lo, hi)
    def permutation(self, n):
        return jax.random.permutation(self._next(), n)


kernel_name = 'standalone__seq2seq_rnn_t_joint__speech'

def setup_inputs():
    _rng = _Rng(jax.random.key(int.from_bytes(__import__("os").urandom(4), "little")))
    _w = (lambda a: (lambda t: t.astype(jnp.bfloat16) if jnp.issubdtype(t.dtype, jnp.floating) else t)(jnp.asarray(a)))
    B, T, D, K = 2, 1000, 512, 31
    U = 8
    sc = (1.0 / (K * D)) ** 0.5
    sd = (1.0 / D) ** 0.5
    return {
        "x": _w((lambda *s: _rng.normal(s) * 0.4)(B, T, D) * 0.5),
        "w1": _w((lambda *s: _rng.normal(s) * 1.6)(K, D, D) * sc),
        "w2": _w((lambda *s: _rng.normal(s) * 1.6)(K, D, D) * sc),
        "g": _w((lambda *s: _rng.normal(s) * 1.6)(B, U, D) * 0.5),
        "w_f": _w((lambda *s: _rng.normal(s) * 1.6)(D, D) * sd),
        "w_g": _w((lambda *s: _rng.normal(s) * 1.6)(D, D) * sd),
        "w_o": _w((lambda *s: _rng.normal(s) * 1.6)(D, D) * sd),
    }

def reference(x, w1, w2, g, w_f, w_g, w_o):
    B, T, D = x.shape
    K = w1.shape[0]
    pad = K // 2
    xp = jnp.pad(x, ((0,0),(pad,pad),(0,0)))
    h = jnp.zeros_like(x)
    for i in range(K):
        h = h + jnp.einsum("btc,cd->btd", xp[:, i:i+T, :], w1[i])
    h = _gelu(h)[:, ::2, :]
    T1 = h.shape[1]
    hp = jnp.pad(h, ((0,0),(pad,pad),(0,0)))
    f = jnp.zeros_like(h)
    for i in range(K):
        f = f + jnp.einsum("btc,cd->btd", hp[:, i:i+T1, :], w2[i])
    f = _gelu(f)[:, ::2, :]
    fe = jnp.einsum("btd,de->bte", f, w_f)
    ge = jnp.einsum("bud,de->bue", g, w_g)
    j = jnp.tanh(fe[:, :, None, :] + ge[:, None, :, :])
    return jnp.einsum("btud,dv->btuv", j, w_o)
```

```python
import functools
import jax
import jax.numpy as jnp
from jax import lax
import jax.experimental.pallas as pl
import jax.experimental.pallas.tpu as pltpu

f32 = jnp.float32
bf16 = jnp.bfloat16
u32 = jnp.uint32

L1 = 3
L2 = 3
KH = 2
CH = 50
FLAGS = None
CUT = 3
ORD = 0


def _digits(L):
    out = [()]
    for _ in range(L):
        out = [c + (d,) for c in out for d in range(3)]
    return out


def _in_tree(L, z):
    memo = {}

    def val(c, o):
        if (c, o) not in memo:
            if not c:
                v = z(o)
            elif c[-1] == 0:
                v = val(c[:-1], 2 * o) - val(c[:-1], 2 * o + 1)
            elif c[-1] == 1:
                v = val(c[:-1], 2 * o + 1)
            else:
                v = val(c[:-1], 2 * o + 2) - val(c[:-1], 2 * o + 1)
            memo[(c, o)] = v
        return memo[(c, o)]
    return [val(c, 0) for c in _digits(L)]


def _w_tree(L, w):
    memo = {}

    def val(c, a):
        if (c, a) not in memo:
            if not c:
                v = w(a)
            elif c[-1] == 0:
                v = val(c[:-1], 2 * a)
            elif c[-1] == 1:
                v = val(c[:-1], 2 * a) + val(c[:-1], 2 * a + 1)
            else:
                v = val(c[:-1], 2 * a + 1)
            memo[(c, a)] = v
        return memo[(c, a)]
    return {c: val(c, 0) for c in _digits(L) if 1 in c}


def _pure_r(c):
    r = 0
    for i, d in enumerate(c):
        r += (d // 2) << i
    return r


def _terms(c):
    rs = [0]
    for i, d in enumerate(c):
        if d == 0:
            pass
        elif d == 2:
            rs = [r + (1 << i) for r in rs]
        else:
            rs = rs + [r + (1 << i) for r in rs]
    return rs


def _parts(c):
    keep = c.index(1)
    out = [()]
    for i, d in enumerate(c):
        if d == 1 and i != keep:
            out = [p + (x,) for p in out for x in (0, 2)]
        else:
            out = [p + (d,) for p in out]
    return out


def _order(L):
    dig = _digits(L)
    by = lambda n: [c for c in dig if len(_terms(c)) == n]
    multi = [c for c in dig if len(_terms(c)) > 2]
    stored = sorted({p for c in multi for p in _parts(c)})
    two = stored + [c for c in by(2) if c not in stored]
    pure = by(1)
    order = []
    for i, c in enumerate(two):
        if i < len(pure) // 2:
            order.append(pure[i])
        order.append(c)
    rest = pure[len(pure) // 2:]
    for i, c in enumerate(multi):
        if i < len(rest):
            order.append(rest[i])
        order.append(c)
    order += rest[len(multi):]
    assert sorted(order) == sorted(dig)
    return order, stored


def _out_tree(L, p):
    memo = {}

    def val(c, q):
        if (c, q) not in memo:
            if len(c) == L:
                v = p(c)
            elif q & 1 == 0:
                v = val(c + (0,), q >> 1) + val(c + (1,), q >> 1)
            else:
                v = val(c + (1,), q >> 1) + val(c + (2,), q >> 1)
            memo[(c, q)] = v
        return memo[(c, q)]
    return [val((), q) for q in range(2 ** L)]


def _gelu(x):
    return jax.nn.gelu(x, approximate=True)


@jax.jit
def pallas_standalone__seq2seq_rnn_t_joint__speech_kernel(x, w1, w2, g, w_f, w_g, w_o):
    B, T, D = x.shape
    K = w1.shape[0]
    U = g.shape[1]
    T1 = (T + 1) // 2
    T2 = (T1 + 1) // 2
    assert (B, T, D, K, U) == (2, 1000, 512, 31, 8)
    KK = D // KH
    LBK = KK // 128
    OFF1 = 520
    OFF2 = OFF1 // 2
    Pn1, Pn2 = 2 ** L1, 2 ** L2
    A1, A2 = 16 // Pn1, 16 // Pn2
    M1, M2 = 1024 // Pn1, 512 // Pn2
    NS1, NS2 = 3 ** L1, 3 ** L2
    NG1, NG2 = A1 * 2 * KH, A2 * 2 * KH
    JR1, JR2 = M1 + 8, M2 + 8
    XR = 1024 + 80
    R = 2 * Pn2 // Pn1
    assert R >= 1
    HOFF = 8
    HR = HOFF + R * JR2 + 16
    dig1, dig2 = _digits(L1), _digits(L2)
    np1 = [c for c in dig1 if 1 in c]
    np2 = [c for c in dig2 if 1 in c]
    NV = max(len(np1), len(np2))
    NCH = T2 // CH

    def kern(x_hbm, w1_hbm, w2_hbm, g_ref, wf_ref, wg_ref, wo_ref, o_hbm,
             xb, S1, P1, hq, S2, P2, W1v, W2v, Tb, fb, ob, sem_x, s1, s2, sem_o):

        def x_copies():
            xh = x_hbm.bitcast(u32)
            return [pltpu.make_async_copy(xh.at[b, :, pl.ds(128 * lb, 128)],
                                          xb.at[lb, pl.ds(8 + OFF1 * b, T // 2), :], sem_x)
                    for b in range(B) for lb in range(4)]

        def w_dma(w_hbm, Wv, sem, Pn, gi, start):
            kh = gi % KH
            ae = gi // KH
            e = ae % 2
            a = ae // 2
            k0 = kh * (KK // 2)
            if not isinstance(gi, int):
                k0 = pl.multiple_of(k0, KK // 2)
            for r in range(Pn):
                i = 2 * (Pn * a + r) + e - 1
                def go(i=i, r=r):
                    cp = pltpu.make_async_copy(w_hbm.bitcast(u32).at[i, pl.ds(k0, KK // 2), :], Wv.at[gi, r], sem.at[gi])
                    if start:
                        cp.start()
                    else:
                        cp.wait()
                if r > 0:
                    go()
                elif isinstance(gi, int):
                    if i >= 0:
                        go()
                else:
                    pl.when(ae > 0)(go)

        NU = (KK // 16) * 4
        def w_transform(L, Wv, gi, V, nps, lo=0, hi=NU):
            for un in range(lo, hi):
                rb, lb = un // 4, un % 4
                if True:
                    sl = (pl.ds(8 * rb, 8), pl.ds(128 * lb, 128))
                    raw = [Wv[(gi, r) + sl] for r in range(2 ** L)]
                    vals = [_w_tree(L, lambda r: pltpu.unpack_elementwise(
                        raw[r], index=h, packed_dtype=bf16, unpacked_dtype=f32)) for h in range(2)]
                    for n, c in enumerate(nps):
                        V[(n,) + sl] = pltpu.bitcast(
                            pltpu.pack_elementwise([vals[0][c], vals[1][c]], packed_dtype=bf16), u32)

        def dots(dig, nps, M, S, P, Wv, gi, V, lo, hi):
            kh = gi % KH
            ae = gi // KH
            e = ae % 2
            a = ae // 2
            order, stored = _order(len(dig[0]))
            for c in order:
                ci = dig.index(c)
                lhs = jnp.concatenate(
                    [S[ci, e, kh * LBK + l, pl.ds(a, M), :] for l in range(LBK)], axis=1).astype(bf16)
                rs = _terms(c)
                if len(rs) == 1:
                    rhs = Wv[gi, rs[0]]
                else:
                    if len(rs) == 2:
                        raw = [Wv[gi, r] for r in rs]
                        hs = []
                        for h in range(2):
                            v = [pltpu.unpack_elementwise(z, index=h, packed_dtype=bf16, unpacked_dtype=f32) for z in raw]
                            hs.append(v[0] + v[1])
                            if c in stored:
                                Tb[stored.index(c), h] = hs[-1]
                    else:
                        hs = []
                        for h in range(2):
                            v = [Tb[stored.index(p), h] for p in _parts(c)]
                            while len(v) > 1:
                                v = [v[2 * i] + v[2 * i + 1] for i in range(len(v) // 2)]
                            hs.append(v[0])
                    rhs = pltpu.bitcast(pltpu.pack_elementwise(hs, packed_dtype=bf16), u32)
                rhs = pltpu.bitcast(rhs, bf16)
                P[ci] += jnp.dot(lhs, rhs, preferred_element_type=f32)

        xc = x_copies()
        for cp in xc:
            cp.start()
        w_dma(w1_hbm, W1v, s1, Pn1, 0, True)
        w_dma(w1_hbm, W1v, s1, Pn1, 1, True)
        for lb in range(4):
            xb[lb, pl.ds(0, 8), :] = jnp.zeros((8, 128), u32)
            xb[lb, pl.ds(8 + T1, OFF1 - T1), :] = jnp.zeros((OFF1 - T1, 128), u32)
            xb[lb, pl.ds(8 + OFF1 + T1, XR - 8 - OFF1 - T1), :] = jnp.zeros((XR - 8 - OFF1 - T1, 128), u32)
        for kh in range(KH):
            W1v[kh, 0] = jnp.zeros((KK // 2, D), u32)
            W2v[kh, 0] = jnp.zeros((KK // 2, D), u32)
        P1[...] = jnp.zeros_like(P1)
        P2[...] = jnp.zeros_like(P2)
        hq[...] = jnp.zeros_like(hq)
        with jax.named_scope('ph_xwait'):
            for cp in xc:
                cp.wait()

        xu = xb

        def in1(jc, carry):
            j0 = pl.multiple_of(jc * 8, 8)
            for lb in range(4):
                zc = {}
                def zload(o):
                    if o not in zc:
                        zc[o] = xu[lb, pl.ds(Pn1 * j0 + o, 8, stride=Pn1), :]
                    return zc[o]
                for e in range(2):
                    if e == 0:
                        z = lambda o: pltpu.bitcast(zload(o) << 16, f32)
                    else:
                        z = lambda o: pltpu.bitcast(zload(o) & u32(0xFFFF0000), f32)
                    vals = _in_tree(L1, z)
                    for ci in range(NS1):
                        S1[ci, e, lb, pl.ds(j0, 8), :] = vals[ci]
            return carry
        with jax.named_scope('ph_in1'):
            lax.fori_loop(0, JR1 // 8, in1, 0)

        with jax.named_scope('ph_w0'):
            pass

        def conv_step(first, gi, Vr, Vw, last_expr):
            if first:
                dig, nps, M, S, P, Wv, NG = dig1, np1, M1, S1, P1, W1v, NG1
            else:
                dig, nps, M, S, P, Wv, NG = dig2, np2, M2, S2, P2, W2v, NG2
            NS = len(dig)
            cut = NS // 3
            dots(dig, nps, M, S, P, Wv, gi, Vr, 0, cut)
            return functools.partial(dots, dig, nps, M, S, P, Wv, gi, Vr, cut, NS)

        def start_global(G):
            if G < NG1:
                w_dma(w1_hbm, W1v, s1, Pn1, G, True)
            elif G < NG1 + NG2:
                w_dma(w2_hbm, W2v, s2, Pn2, G - NG1, True)

        def conv_loop(first):
            NG = NG1 if first else NG2
            if first:
                w_hbm, Wv, sem, Pn, L, nps = w1_hbm, W1v, s1, Pn1, L1, np1
            else:
                w_hbm, Wv, sem, Pn, L, nps = w2_hbm, W2v, s2, Pn2, L2, np2

            dig, M, S, P = (dig1, M1, S1, P1) if first else (dig2, M2, S2, P2)
            def body(gi, carry):
                w_dma(w_hbm, Wv, sem, Pn, gi, False)
                @pl.when(gi + 2 < NG)
                def _():
                    w_dma(w_hbm, Wv, sem, Pn, gi + 2, True)
                if first:
                    @pl.when(gi + 2 >= NG)
                    def _():
                        w_dma(w2_hbm, W2v, s2, Pn2, gi + 2 - NG, True)
                dots(dig, nps, M, S, P, Wv, gi, None, 0, len(dig))
                return carry
            lax.fori_loop(0, NG, body, 0)

        with jax.named_scope('ph_conv1'):
            conv_loop(True)

        def out1(sc, carry):
            s0 = pl.multiple_of(sc * 8, 8)
            srow = s0 + lax.broadcasted_iota(jnp.int32, (8, 128), 0)
            for lb in range(4):
                ys = _out_tree(L1, lambda c: P1[dig1.index(c), pl.ds(s0, 8), pl.ds(128 * lb, 128)])
                for q in range(Pn1):
                    t = Pn1 * srow + q
                    valid = (t < T1) | ((t >= OFF1) & (t < OFF1 + T1))
                    hq[q, lb, pl.ds(HOFF + s0, 8), :] = jnp.where(valid, _gelu(ys[q]), 0.0)
            return carry
        with jax.named_scope('ph_out1'):
            lax.fori_loop(0, M1 // 8, out1, 0)

        def in2(jc, carry):
            j0 = pl.multiple_of(jc * 8, 8)
            for lb in range(4):
                for e in range(2):
                    def z(o):
                        n = 2 * o + e - 16
                        q, so = n % Pn1, n // Pn1
                        if R == 1:
                            return hq[q, lb, pl.ds(HOFF + so + j0, 8), :]
                        return hq[q, lb, pl.ds(HOFF + so + R * j0, 8, stride=R), :]
                    vals = _in_tree(L2, z)
                    for ci in range(NS2):
                        S2[ci, e, lb, pl.ds(j0, 8), :] = vals[ci]
            return carry
        with jax.named_scope('ph_in2'):
            lax.fori_loop(0, JR2 // 8, in2, 0)

        with jax.named_scope('ph_conv2'):
            conv_loop(False)

        def out2(sc, carry):
            s0 = pl.multiple_of(sc * 8, 8)
            for lb in range(4):
                ys = _out_tree(L2, lambda c: P2[dig2.index(c), pl.ds(s0, 8), pl.ds(128 * lb, 128)])
                for q in range(Pn2):
                    fb[lb, pl.ds(Pn2 * s0 + q, 8, stride=Pn2), :] = _gelu(ys[q])
            return carry
        with jax.named_scope('ph_out2'):
            lax.fori_loop(0, M2 // 8, out2, 0)

        fl = jnp.concatenate([fb[lb] for lb in range(4)], axis=1).astype(bf16)
        fe = jnp.dot(fl, wf_ref[...], preferred_element_type=f32)
        for lb in range(4):
            fb[lb] = fe[:, 128 * lb:128 * (lb + 1)]
        ge = jnp.dot(g_ref[...], wg_ref[...], preferred_element_type=f32)

        def o_copy(b, ch):
            return pltpu.make_async_copy(ob.at[b * NCH + ch], o_hbm.at[pl.ds((b * NCH + ch) * CH * U, CH * U), :],
                                         sem_o.at[b * NCH + ch])
        for b in range(B):
            geb = ge[b * U:(b + 1) * U]
            def jbody(ch, carry):
                t0 = OFF2 * b + ch * CH
                fr = jnp.concatenate([fb[lb, pl.ds(t0, CH), :] for lb in range(4)], axis=1)
                j = jnp.tanh(fr[:, None, :] + geb[None, :, :]).reshape(CH * U, D).astype(bf16)
                ob[b * NCH + ch] = jnp.dot(j, wo_ref[...], preferred_element_type=f32).astype(bf16)
                o_copy(b, ch).start()
                return carry
            with jax.named_scope('ph_joint'):
                lax.fori_loop(0, NCH, jbody, 0)
        with jax.named_scope('ph_owait'):
            for b in range(B):
                for ch in range(NCH):
                    o_copy(b, ch).wait()

    vm = pl.BlockSpec(memory_space=pltpu.VMEM)
    hb = pl.BlockSpec(memory_space=pl.ANY)
    out = pl.pallas_call(
        kern,
        out_shape=jax.ShapeDtypeStruct((B * T2 * U, D), bf16),
        in_specs=[hb, hb, hb, vm, vm, vm, vm],
        out_specs=hb,
        scratch_shapes=[
            pltpu.VMEM((4, XR, 128), u32),
            pltpu.VMEM((NS1, 2, 4, JR1, 128), f32), pltpu.VMEM((NS1, M1, D), f32),
            pltpu.VMEM((Pn1, 4, HR, 128), f32),
            pltpu.VMEM((NS2, 2, 4, JR2, 128), f32), pltpu.VMEM((NS2, M2, D), f32),
            pltpu.VMEM((NG1, Pn1, KK // 2, D), u32), pltpu.VMEM((NG2, Pn2, KK // 2, D), u32),

            pltpu.VMEM((8, 2, KK // 2, D), f32),
            pltpu.VMEM((4, 512, 128), f32),
            pltpu.VMEM((B * NCH, CH * U, D), bf16),
            pltpu.SemaphoreType.DMA, pltpu.SemaphoreType.DMA((NG1,)), pltpu.SemaphoreType.DMA((NG2,)),
            pltpu.SemaphoreType.DMA((B * NCH,)),
        ],
        compiler_params=pltpu.CompilerParams(vmem_limit_bytes=110 * 1024 * 1024, flags=FLAGS),
    )(x, w1, w2, g.reshape(B * U, D), w_f, w_g, w_o)
    return out.reshape(B, T2, U, D)
```

```python
import functools
import jax
import jax.numpy as jnp
from jax import lax
import jax.experimental.pallas as pl
import jax.experimental.pallas.tpu as pltpu

f32 = jnp.float32
bf16 = jnp.bfloat16
u32 = jnp.uint32

L1 = 3
L2 = 3
KH1 = 2
KH2 = 1
CH = 50


def _digits(L):
    out = [()]
    for _ in range(L):
        out = [c + (d,) for c in out for d in range(3)]
    return out


def _in_tree(L, z):
    memo = {}

    def val(c, o):
        if (c, o) not in memo:
            if not c:
                v = z(o)
            elif c[-1] == 0:
                v = val(c[:-1], 2 * o) - val(c[:-1], 2 * o + 1)
            elif c[-1] == 1:
                v = val(c[:-1], 2 * o + 1)
            else:
                v = val(c[:-1], 2 * o + 2) - val(c[:-1], 2 * o + 1)
            memo[(c, o)] = v
        return memo[(c, o)]
    return [val(c, 0) for c in _digits(L)]


def _terms(c):
    rs = [0]
    for i, d in enumerate(c):
        if d == 0:
            pass
        elif d == 2:
            rs = [r + (1 << i) for r in rs]
        else:
            rs = rs + [r + (1 << i) for r in rs]
    return rs


def _parts(c):
    keep = c.index(1)
    out = [()]
    for i, d in enumerate(c):
        if d == 1 and i != keep:
            out = [p + (x,) for p in out for x in (0, 2)]
        else:
            out = [p + (d,) for p in out]
    return out


def _order(L):
    dig = _digits(L)
    by = lambda n: [c for c in dig if len(_terms(c)) == n]
    multi = [c for c in dig if len(_terms(c)) > 2]
    stored = sorted({p for c in multi for p in _parts(c)})
    two = stored + [c for c in by(2) if c not in stored]
    pure = by(1)
    order = []
    for i, c in enumerate(two):
        if i < len(pure) // 2:
            order.append(pure[i])
        order.append(c)
    rest = pure[len(pure) // 2:]
    for i, c in enumerate(multi):
        if i < len(rest):
            order.append(rest[i])
        order.append(c)
    order += rest[len(multi):]
    assert sorted(order) == sorted(dig)
    return order, stored


def _out_tree(L, p):
    memo = {}

    def val(c, q):
        if (c, q) not in memo:
            if len(c) == L:
                v = p(c)
            elif q & 1 == 0:
                v = val(c + (0,), q >> 1) + val(c + (1,), q >> 1)
            else:
                v = val(c + (1,), q >> 1) + val(c + (2,), q >> 1)
            memo[(c, q)] = v
        return memo[(c, q)]
    return [val((), q) for q in range(2 ** L)]


def _pack(lo, hi):
    return pltpu.bitcast(pltpu.pack_elementwise([lo, hi], packed_dtype=bf16), u32)


def _gelu(x):
    return jax.nn.gelu(x, approximate=True)


@jax.jit
def pallas_standalone__seq2seq_rnn_t_joint__speech_kernel(x, w1, w2, g, w_f, w_g, w_o):
    B, T, D = x.shape
    K = w1.shape[0]
    U = g.shape[1]
    T1 = (T + 1) // 2
    T2 = (T1 + 1) // 2
    assert (B, T, D, K, U) == (2, 1000, 512, 31, 8)
    OFF1 = 520
    OFF2 = OFF1 // 2
    Pn1, Pn2 = 2 ** L1, 2 ** L2
    A1, A2 = 16 // Pn1, 16 // Pn2
    M1, M2 = 1024 // Pn1, 512 // Pn2
    NS1, NS2 = 3 ** L1, 3 ** L2
    NG1, NG2 = A1 * 2 * KH1, A2 * 2 * KH2
    KK1, KK2 = D // KH1, D // KH2
    H1, H2 = M1 // 2, M2 // 2
    JR1, JR2 = H1 + 8, H2 + 8
    XR = 1024 + 80
    R = 2 * Pn2 // Pn1
    assert R >= 1
    HOFF = 8
    HR = HOFF + R * (H2 + JR2) + 16
    assert Pn1 * (H1 + JR1 + 1) <= XR
    dig1, dig2 = _digits(L1), _digits(L2)
    NCH = T2 // CH

    def kern(x_hbm, w1_hbm, w2_hbm, g_hbm, wf_hbm, wg_hbm, wo_hbm, o_hbm,
             xb, S1, P1, hq, S2, P2, W1v, W2v, Tb, fb, ob, gv, wfv, wgv, wov,
             sem_x, s1, s2, sem_o, sem_m):

        def x_copies(half):
            xh = x_hbm.bitcast(u32)
            return [pltpu.make_async_copy(xh.at[b, :, pl.ds(128 * lb, 128)],
                                          xb.at[lb, pl.ds(8 + OFF1 * b, T // 2), :], sem_x.at[half])
                    for lb in (2 * half, 2 * half + 1) for b in range(B)]

        misc = [pltpu.make_async_copy(g_hbm, gv, sem_m.at[0]),
                pltpu.make_async_copy(wf_hbm.bitcast(u32), wfv, sem_m.at[1]),
                pltpu.make_async_copy(wg_hbm.bitcast(u32), wgv, sem_m.at[2]),
                pltpu.make_async_copy(wo_hbm.bitcast(u32), wov, sem_m.at[3])]

        w1h, w2h = w1_hbm.bitcast(u32), w2_hbm.bitcast(u32)

        def w_small(gi):
            kh, e = gi % KH1, gi // KH1
            ks = pl.ds(kh * (KK1 // 2), KK1 // 2)
            return [pltpu.make_async_copy(w1h.at[2 * r + e - 1, ks, :], W1v.at[2 * r + e, ks, :], s1.at[gi])
                    for r in range(Pn1) if 2 * r + e >= 1]
        NSM = 2 * KH1
        big1 = pltpu.make_async_copy(w1h.at[pl.ds(2 * Pn1 - 1, 32 - 2 * Pn1)], W1v.at[pl.ds(2 * Pn1, 32 - 2 * Pn1)], s1.at[NSM])
        big2 = pltpu.make_async_copy(w2h, W2v.at[pl.ds(1, 31)], s2.at[0])

        def dots(first, gi):
            dig, M, S, P, Wv, KH, KK = ((dig1, M1, S1, P1, W1v, KH1, KK1) if first
                                        else (dig2, M2, S2, P2, W2v, KH2, KK2))
            LBK = KK // 128
            kh = gi % KH
            ae = gi // KH
            e = ae % 2
            a = ae // 2
            order, stored = _order(len(dig[0]))
            Pn = 2 ** len(dig[0])
            ks = pl.ds(kh * (KK // 2) if KH == 1 else pl.multiple_of(kh * (KK // 2), KK // 2), KK // 2)
            tap = lambda r: Wv[2 * (Pn * a + r) + e, ks, :]
            for c in order:
                ci = dig.index(c)
                lhs = pltpu.bitcast(jnp.concatenate(
                    [S[ci, e, kh * LBK + l, pl.ds(a, M // 2), :] for l in range(LBK)], axis=1), bf16)
                rs = _terms(c)
                if len(rs) == 1:
                    rhs = tap(rs[0])
                else:
                    hs = []
                    if len(rs) == 2:
                        raw = [tap(r) for r in rs]
                        for h in range(2):
                            v = [pltpu.unpack_elementwise(z, index=h, packed_dtype=bf16, unpacked_dtype=f32) for z in raw]
                            hs.append(v[0] + v[1])
                            if c in stored:
                                Tb[stored.index(c), h, pl.ds(0, KK // 2), :] = hs[-1]
                    else:
                        for h in range(2):
                            v = [Tb[stored.index(p), h, pl.ds(0, KK // 2), :] for p in _parts(c)]
                            while len(v) > 1:
                                v = [v[2 * i] + v[2 * i + 1] for i in range(len(v) // 2)]
                            hs.append(v[0])
                    rhs = pltpu.bitcast(pltpu.pack_elementwise(hs, packed_dtype=bf16), u32)
                rhs = pltpu.bitcast(rhs, bf16)
                r = jnp.dot(lhs, rhs, preferred_element_type=f32)
                for lb in range(4):
                    P[ci, lb] += r[:, 128 * lb:128 * (lb + 1)]

        xc = [x_copies(0), x_copies(1)]
        for cp in xc[0] + xc[1]:
            cp.start()
        for cp in w_small(0):
            cp.start()
        for lb in range(4):
            xb[lb, pl.ds(0, 8), :] = jnp.zeros((8, 128), u32)
            xb[lb, pl.ds(8 + T1, OFF1 - T1), :] = jnp.zeros((OFF1 - T1, 128), u32)
            xb[lb, pl.ds(8 + OFF1 + T1, XR - 8 - OFF1 - T1), :] = jnp.zeros((XR - 8 - OFF1 - T1, 128), u32)
        W1v[0] = jnp.zeros((D // 2, D), u32)
        W2v[0] = jnp.zeros((D // 2, D), u32)
        P1[...] = jnp.zeros_like(P1)
        hq[:, :, pl.ds(0, HOFF), :] = jnp.zeros((Pn1, 4, HOFF, 128), f32)
        hq[:, :, pl.ds(HOFF + M1, HR - HOFF - M1), :] = jnp.zeros((Pn1, 4, HR - HOFF - M1, 128), f32)

        def in1(half, jc, carry):
            j0 = pl.multiple_of(jc * 8, 8)
            for lb in (2 * half, 2 * half + 1):
                zc = {}
                def zload(h, o):
                    if (h, o) not in zc:
                        zc[h, o] = xb[lb, pl.ds(Pn1 * (j0 + h * H1) + o, 8, stride=Pn1), :]
                    return zc[h, o]
                for e in range(2):
                    vals = []
                    for h in range(2):
                        if e == 0:
                            z = lambda o: pltpu.bitcast(zload(h, o) << 16, f32)
                        else:
                            z = lambda o: pltpu.bitcast(zload(h, o) & u32(0xFFFF0000), f32)
                        vals.append(_in_tree(L1, z))
                    for ci in range(NS1):
                        S1[ci, e, lb, pl.ds(j0, 8), :] = _pack(vals[0][ci], vals[1][ci])
            return carry
        for half in range(2):
            with jax.named_scope('ph_xwait'):
                for cp in xc[half]:
                    cp.wait()
            if half == 0:
                for cp in w_small(1):
                    cp.start()
            with jax.named_scope('ph_in1'):
                lax.fori_loop(0, JR1 // 8, functools.partial(in1, half), 0)

        with jax.named_scope('ph_conv1'):
            def body(gi, carry):
                for k in range(NSM + 1):
                    @pl.when(gi == k)
                    def _():
                        for cp in (w_small(k) if k < NSM else [big1]):
                            cp.wait()
                        if k == 0:
                            for cp in w_small(2) + w_small(3):
                                cp.start()
                        elif k == 1:
                            big1.start()
                        elif k == 3:
                            big2.start()
                dots(True, gi)
                return carry
            lax.fori_loop(0, NG1, body, 0)
        for cp in misc:
            cp.start()

        def out1(sc, carry):
            s0 = pl.multiple_of(sc * 8, 8)
            r0 = 2 * (s0 % H1) + s0 // H1
            srow = s0 + lax.broadcasted_iota(jnp.int32, (8, 128), 0)
            if M2 * 2 == M1:
                for ci in range(NS2):
                    for lb in range(2):
                        P2[ci, 2 * (s0 // M2) + lb, pl.ds(pl.multiple_of(s0 % M2, 8), 8), :] = jnp.zeros((8, 128), f32)
            for lb in range(4):
                ys = _out_tree(L1, lambda c: P1[dig1.index(c), lb, pl.ds(r0, 8, stride=2), :])
                for q in range(Pn1):
                    t = Pn1 * srow + q
                    valid = (t < T1) | ((t >= OFF1) & (t < OFF1 + T1))
                    hq[q, lb, pl.ds(HOFF + s0, 8), :] = jnp.where(valid, _gelu(ys[q]), 0.0)
            return carry
        with jax.named_scope('ph_out1'):
            lax.fori_loop(0, M1 // 8, out1, 0)

        def in2(jc, carry):
            j0 = pl.multiple_of(jc * 8, 8)
            for lb in range(4):
                for e in range(2):
                    vals = []
                    for h in range(2):
                        def z(o):
                            n = 2 * o + e - 16
                            q, so = n % Pn1, n // Pn1
                            return hq[q, lb, pl.ds(HOFF + so + R * (j0 + h * H2), 8, stride=R), :]
                        vals.append(_in_tree(L2, z))
                    for ci in range(NS2):
                        S2[ci, e, lb, pl.ds(j0, 8), :] = _pack(vals[0][ci], vals[1][ci])
            return carry
        with jax.named_scope('ph_in2'):
            lax.fori_loop(0, JR2 // 8, in2, 0)

        with jax.named_scope('ph_conv2'):
            big2.wait()
            def body2(gi, carry):
                dots(False, gi)
                return carry
            lax.fori_loop(0, NG2, body2, 0)

        def out2(sc, carry):
            s0 = pl.multiple_of(sc * 8, 8)
            r0 = 2 * (s0 % H2) + s0 // H2
            for lb in range(4):
                ys = _out_tree(L2, lambda c: P2[dig2.index(c), lb, pl.ds(r0, 8, stride=2), :])
                for q in range(Pn2):
                    fb[lb, pl.ds(Pn2 * s0 + q, 8, stride=Pn2), :] = _gelu(ys[q])
            return carry
        with jax.named_scope('ph_out2'):
            lax.fori_loop(0, M2 // 8, out2, 0)

        for cp in misc:
            cp.wait()
        with jax.named_scope('ph_fe'):
            fl = jnp.concatenate([fb[lb] for lb in range(4)], axis=1).astype(bf16)
            fe = jnp.dot(fl, pltpu.bitcast(wfv[...], bf16), preferred_element_type=f32)
            for lb in range(4):
                fb[lb] = fe[:, 128 * lb:128 * (lb + 1)]
            ge = jnp.dot(gv[...], pltpu.bitcast(wgv[...], bf16), preferred_element_type=f32)

        def o_copy(b, ch):
            return pltpu.make_async_copy(ob.at[b * NCH + ch], o_hbm.at[pl.ds((b * NCH + ch) * CH * U, CH * U), :],
                                         sem_o.at[b * NCH + ch])
        with jax.named_scope('ph_joint'):
            for b in range(B):
                geb = ge[b * U:(b + 1) * U]
                def jbody(ch, carry):
                    t0 = OFF2 * b + ch * CH
                    fr = jnp.concatenate([fb[lb, pl.ds(t0, CH), :] for lb in range(4)], axis=1)
                    j = jnp.tanh(fr[:, None, :] + geb[None, :, :]).reshape(CH * U, D).astype(bf16)
                    ob[b * NCH + ch] = jnp.dot(j, pltpu.bitcast(wov[...], bf16), preferred_element_type=f32).astype(bf16)
                    o_copy(b, ch).start()
                    return carry
                for ch in range(NCH):
                    jbody(ch, 0)
        with jax.named_scope('ph_owait'):
            for b in range(B):
                for ch in range(NCH):
                    o_copy(b, ch).wait()

    hb = pl.BlockSpec(memory_space=pl.ANY)
    out = pl.pallas_call(
        kern,
        out_shape=jax.ShapeDtypeStruct((B * T2 * U, D), bf16),
        in_specs=[hb] * 7,
        out_specs=hb,
        scratch_shapes=[
            pltpu.VMEM((4, XR, 128), u32),
            pltpu.VMEM((NS1, 2, 4, JR1, 128), u32), pltpu.VMEM((NS1, 4, M1, 128), f32),
            pltpu.VMEM((Pn1, 4, HR, 128), f32),
            pltpu.VMEM((NS2, 2, 4, JR2, 128), u32), pltpu.VMEM((NS2, 4, M2, 128), f32),
            pltpu.VMEM((32, D // 2, D), u32), pltpu.VMEM((32, D // 2, D), u32),
            pltpu.VMEM((8, 2, max(KK1, KK2) // 2, D), f32),
            pltpu.VMEM((4, 512, 128), f32),
            pltpu.VMEM((B * NCH, CH * U, D), bf16),
            pltpu.VMEM((B * U, D), bf16),
            pltpu.VMEM((D // 2, D), u32), pltpu.VMEM((D // 2, D), u32), pltpu.VMEM((D // 2, D), u32),
            pltpu.SemaphoreType.DMA((2,)), pltpu.SemaphoreType.DMA((NG1,)), pltpu.SemaphoreType.DMA((NG2,)),
            pltpu.SemaphoreType.DMA((B * NCH,)), pltpu.SemaphoreType.DMA((4,)),
        ],
        compiler_params=pltpu.CompilerParams(vmem_limit_bytes=110 * 1024 * 1024),
    )(x, w1, w2, g.reshape(B * U, D), w_f, w_g, w_o)
    return out.reshape(B, T2, U, D)
```
